```python
import jax
import jax.numpy as jnp

def _softmax(x, axis=-1):
    return jax.nn.softmax(x, axis=axis)
def _gelu(x):
    return jax.nn.gelu(x, approximate=True)
def _silu(x):
    return jax.nn.silu(x)
def _sigmoid(x):
    return jax.nn.sigmoid(x)
def _layernorm(x, axis=-1, eps=1e-5):
    m = jnp.mean(x, axis=axis, keepdims=True)
    v = jnp.var(x, axis=axis, keepdims=True)
    return (x - m) / jnp.sqrt(v + eps)
def _scatter_add(tgt, idx, src, axis=0):
    return tgt.at[idx].add(src)
def _segment_sum(src, seg, n):
    return jax.ops.segment_sum(src, seg, n)
class _Rng:
    def __init__(self, key):
        self._k = key
    def _next(self):
        self._k, sub = jax.random.split(self._k)
        return sub
    def normal(self, shape):
        return jax.random.normal(self._next(), shape, dtype=jnp.bfloat16)
    def randint(self, lo, hi, shape):
        return jax.random.randint(self._next(), shape, lo, hi, dtype=jnp.int32)
    def uniform(self, shape, lo=0.0, hi=1.0):
        return jax.random.uniform(self._next(), shape, jnp.bfloat16, lo, hi)
    def permutation(self, n):
        return jax.random.permutation(self._next(), n)


kernel_name = 'gated_mix__sliding_block_cached__moe_arch_mod__decode'

def setup_inputs():
    _rng = _Rng(jax.random.key(int.from_bytes(__import__("os").urandom(4), "little")))
    _w = (lambda a: (lambda t: t.astype(jnp.bfloat16) if jnp.issubdtype(t.dtype, jnp.floating) else t)(jnp.asarray(a)))
    def _A_setup():
        B, Sq, D = 1, 1, 640
        Hq, Hkv, Sk, Dh = 32, 32, 32768, 192
        assert Hq % Hkv == 0, (Hq, Hkv)
        return {
            "x": _w((lambda *s: _rng.normal(s) * 0.05)(B, Sq, D)),
            "k_cache": _w((lambda *s: _rng.normal(s) * 0.05)(B, Hkv, Sk, Dh)),
            "v_cache": _w((lambda *s: _rng.normal(s) * 0.05)(B, Hkv, Sk, Dh)),
            "wq": _w((lambda *s: _rng.normal(s) * 0.05)(D, Hq * Dh) * (D ** -0.5)),
            "wo": _w((lambda *s: _rng.normal(s) * 0.05)(Hq * Dh, D) * ((Hq * Dh) ** -0.5)),
        }
    _A_in = _A_setup()

    def _B_setup():
        B, S, D, F, C = 1, 1, 640, 1536, 1
        return {
            "x": _w((lambda *s: _rng.normal(s) * 0.05)(B, S, D)),
            "w_r": _w((lambda *s: _rng.normal(s) * 0.05)(D)),
            "w_gate": _w((lambda *s: _rng.normal(s) * 0.05)(D, F)),
            "w_up": _w((lambda *s: _rng.normal(s) * 0.05)(D, F)),
            "w_down": _w((lambda *s: _rng.normal(s) * 0.05)(F, D)),
        }
    _B_in = _B_setup()

    return {
        "A_x": _A_in["x"],
        "A_k_cache": _A_in["k_cache"],
        "A_v_cache": _A_in["v_cache"],
        "A_wq": _A_in["wq"],
        "A_wo": _A_in["wo"],
        "B_x": _B_in["x"],
        "B_w_r": _B_in["w_r"],
        "B_w_gate": _B_in["w_gate"],
        "B_w_up": _B_in["w_up"],
        "B_w_down": _B_in["w_down"],
        "gate_w": _w((lambda *s: _rng.normal(s) * 0.05)(640)),
    }

def reference(A_x, A_k_cache, A_v_cache, A_wq, A_wo, B_x, B_w_r, B_w_gate, B_w_up, B_w_down, gate_w):
    def _A_ref(x, k_cache, v_cache, wq, wo):
        B, Sq, D = x.shape
        Hq, Dh = 32, 192
        Hkv, Sk = k_cache.shape[1], k_cache.shape[2]
        W = min(4096, max(256, Sk // 4))
        rep = Hq // Hkv
        q = (lambda x, *d: x.transpose(*d))((x @ wq).reshape(B, Sq, Hq, Dh), 0, 2, 1, 3)
        k = jnp.repeat(k_cache[:, :, Sk - W:, :], rep, axis=1)
        v = jnp.repeat(v_cache[:, :, Sk - W:, :], rep, axis=1)
        scores = jnp.einsum("bhqd,bhkd->bhqk", q, k) * (Dh ** -0.5)
        p = _softmax(scores, axis=-1)
        o = jnp.einsum("bhqk,bhkd->bhqd", p, v)
        return (lambda x, *d: x.transpose(*d))(o, 0, 2, 1, 3).reshape(B, Sq, Hq * Dh) @ wo

    def _B_ref(x, w_r, w_gate, w_up, w_down):
        B, S, D = x.shape
        C = 1
        r = x @ w_r
        idx = jnp.argsort(-r, axis=-1)[:, :C]
        idx_e = jnp.repeat(idx.reshape(B, C, 1), D, axis=2)
        x_sel = jnp.take_along_axis(x, idx_e, axis=1)
        g = _silu(x_sel @ w_gate)
        u = x_sel @ w_up
        y = (g * u) @ w_down
        r_sel = _sigmoid(jnp.take_along_axis(r, idx, axis=1))
        y = y * r_sel.reshape(B, C, 1)
        b_off = (jnp.arange(B) * S).reshape(B, 1)
        flat_idx = (idx + b_off).reshape(B * C)
        zero = (x * 0.0).reshape(B * S, D)
        upd = _scatter_add(zero, flat_idx, y.reshape(B * C, D), axis=0)
        return x + upd.reshape(B, S, D)

    x = A_x
    g = _sigmoid((x * gate_w).sum(-1, keepdims=True))
    a = _A_ref(x, A_k_cache, A_v_cache, A_wq, A_wo)
    b = _B_ref(x, B_w_r, B_w_gate, B_w_up, B_w_down)
    return g * a + (1 - g) * b
```

```python
import functools

import jax
import jax.numpy as jnp
from jax import lax
import jax.experimental.pallas as pl
import jax.experimental.pallas.tpu as pltpu

_HQ = 32
_DH = 192
_G = 2
_PR = _G * _DH
_BAND = 8

_HI, _LO = 0, 1


def _kv_pieces(w, split):
    out = []
    for r in range(0, _PR, _BAND):
        out.append((r, _BAND, 0, split, _HI))
        out.append((r, _BAND, split, w - split, _LO))
    return out


def _w_pieces(nrows, ncols, rows, cols):
    out = []
    j = 0
    for c in range(0, ncols, cols):
        for r in range(0, nrows, rows):
            out.append((r, rows, c, min(cols, ncols - c), _HI if j % 2 == 0 else _LO))
            j += 1
    return out


def _kernel(x_hbm, k_hbm, v_hbm, wq_hbm, wo_hbm, wr_hbm, wg_hbm, wu_hbm, wd_hbm, gw_hbm,
            out_ref,
            x_buf, wr_buf, gw_buf, wq_buf, wo_buf, wg_buf, wu_buf, wd_buf,
            kbuf, vbuf, q_sc, o_sc,
            sem_small, sem_w, sem_k, sem_v, sem_wo,
            *, sk, w, split, wo_chunks):
    d = x_buf.shape[-1]
    npair = _HQ // _G
    c0 = sk - w
    scale = _DH ** -0.5
    f32, bf16 = jnp.float32, jnp.bfloat16

    def start_pieces(src, dst, sem, pieces, row_off=0, col_off=0):
        for (r, nr, c, nc, p) in pieces:
            pltpu.make_async_copy(
                src.at[pl.ds(row_off + r, nr), pl.ds(col_off + c, nc)],
                dst.at[pl.ds(r, nr), pl.ds(c, nc)], sem).start(priority=p)

    def wait_full(dst, sem):
        pltpu.make_async_copy(dst, dst, sem).wait()

    kvp = _kv_pieces(w, split)

    def start_kv(src, buf, sem, pair, slot):
        row = pair * _PR
        if not isinstance(pair, int):
            row = pl.multiple_of(row, _PR)
        start_pieces(src, buf.at[slot], sem.at[slot], kvp, row_off=row, col_off=c0)

    small = [pltpu.make_async_copy(x_hbm, x_buf, sem_small.at[0]),
             pltpu.make_async_copy(wr_hbm, wr_buf, sem_small.at[1]),
             pltpu.make_async_copy(gw_hbm, gw_buf, sem_small.at[2])]
    for cp in small:
        cp.start(priority=_HI)
    start_pieces(wq_hbm, wq_buf, sem_w.at[0], _w_pieces(d, _HQ * _DH, 16, 1024))
    start_pieces(wg_hbm, wg_buf, sem_w.at[1], _w_pieces(d, wg_buf.shape[1], 16, 768))
    start_pieces(wu_hbm, wu_buf, sem_w.at[2], _w_pieces(d, wu_buf.shape[1], 16, 768))
    start_pieces(wd_hbm, wd_buf, sem_w.at[3], _w_pieces(wd_buf.shape[0], d, 16, d))
    start_kv(k_hbm, kbuf, sem_k, 0, 0)

    for cp in small:
        cp.wait()
    x_row = x_buf[0]
    x8 = jnp.broadcast_to(x_row.astype(f32), (8, d)).astype(bf16)

    wait_full(wq_buf, sem_w.at[0])
    q = jnp.dot(x8, wq_buf[...], preferred_element_type=f32)
    row = lax.broadcasted_iota(jnp.int32, q.shape, 0)
    col = lax.broadcasted_iota(jnp.int32, q.shape, 1)
    diag = (col // _DH) % _G == row
    q_sc[...] = jnp.where(diag, q, 0.0)

    start_kv(v_hbm, vbuf, sem_v, 0, 0)

    wait_full(wg_buf, sem_w.at[1])
    wait_full(wu_buf, sem_w.at[2])
    hg = jnp.dot(x8, wg_buf[...], preferred_element_type=f32).astype(bf16).astype(f32)
    hu = jnp.dot(x8, wu_buf[...], preferred_element_type=f32).astype(bf16).astype(f32)
    hact = (hg * jax.nn.sigmoid(hg) * hu).astype(bf16)
    wait_full(wd_buf, sem_w.at[3])
    y = jnp.dot(hact, wd_buf[...], preferred_element_type=f32)[0:1]

    xf = x_row.astype(f32)
    wr = wr_buf[...].astype(f32)
    gw = gw_buf[...].astype(f32)
    nl = d // 128
    racc = sum(xf[:, i * 128:(i + 1) * 128] * wr[i:i + 1, :] for i in range(nl))
    gacc = sum(xf[:, i * 128:(i + 1) * 128] * gw[i:i + 1, :] for i in range(nl))
    r_sel = jax.nn.sigmoid(jnp.sum(racc, axis=1, keepdims=True))
    gate = jax.nn.sigmoid(jnp.sum(gacc, axis=1, keepdims=True))
    b_branch = xf + (xf * 0.0 + y * r_sel)

    orow = lax.broadcasted_iota(jnp.int32, (8, _PR), 0)
    ocol = lax.broadcasted_iota(jnp.int32, (8, _PR), 1)
    odiag = ocol // _DH == orow

    def attend(pair, slot, issue_a, issue_b):
        off = pair * _PR
        if not isinstance(pair, int):
            off = pl.multiple_of(off, 128)
        issue_a()
        wait_full(kbuf.at[slot], sem_k.at[slot])
        qp = q_sc[:, pl.ds(off, _PR)].astype(bf16)
        s = jnp.dot(qp, kbuf[slot], preferred_element_type=f32)
        m = jnp.max(s, axis=1, keepdims=True)
        p = jnp.exp((s - m) * scale)
        l = jnp.sum(p, axis=1, keepdims=True)
        pb = p.astype(bf16)
        issue_b()
        wait_full(vbuf.at[slot], sem_v.at[slot])
        o = lax.dot_general(pb, vbuf[slot], (((1,), (1,)), ((), ())),
                            preferred_element_type=f32)
        o_sc[:, pl.ds(off, _PR)] = jnp.where(odiag, o / l, 0.0)

    def body(pair, carry):
        slot = pair % 2
        nxt = 1 - slot
        attend(pair, slot,
               lambda: start_kv(k_hbm, kbuf, sem_k, pair + 1, nxt),
               lambda: start_kv(v_hbm, vbuf, sem_v, pair + 1, nxt))
        return carry

    lax.fori_loop(0, npair - 1, body, 0)

    def start_wo(i):
        r0, nr = wo_chunks[i]
        start_pieces(wo_hbm, wo_buf.at[pl.ds(r0, nr)], sem_wo.at[i],
                     _w_pieces(nr, d, 16, d), row_off=r0)

    nwo = len(wo_chunks)
    attend(npair - 1, (npair - 1) % 2,
           lambda: start_wo(0),
           lambda: [start_wo(i) for i in range(1, nwo)])

    acc = jnp.zeros((8, d), f32)
    for i, (r0, nr) in enumerate(wo_chunks):
        wait_full(wo_buf.at[pl.ds(r0, nr)], sem_wo.at[i])
        acc = acc + jnp.dot(o_sc[:, r0:r0 + nr].astype(bf16), wo_buf[r0:r0 + nr, :],
                            preferred_element_type=f32)
    a_branch = jnp.sum(acc, axis=0, keepdims=True)
    out_ref[0] = (gate * a_branch + (1.0 - gate) * b_branch).astype(out_ref.dtype)


def _build(A_x, A_k_cache, A_v_cache, A_wq, A_wo, B_w_r, B_w_gate, B_w_up, B_w_down, gate_w,
           split=1152, wo_chunks=((0, 2560), (2560, 2560), (5120, 768), (5888, 256))):
    _, _, d = A_x.shape
    _, hkv, sk, dh = A_k_cache.shape
    assert hkv == _HQ and dh == _DH
    f = B_w_gate.shape[1]
    w = min(4096, max(256, sk // 4))
    kt = jnp.swapaxes(A_k_cache, 2, 3).reshape(_HQ * _DH, sk)
    vt = jnp.swapaxes(A_v_cache, 2, 3).reshape(_HQ * _DH, sk)
    wr = B_w_r.reshape(d // 128, 128)
    gw = gate_w.reshape(d // 128, 128)
    bf16 = jnp.bfloat16
    any_spec = pl.BlockSpec(memory_space=pl.ANY)
    return pl.pallas_call(
        functools.partial(_kernel, sk=sk, w=w, split=split, wo_chunks=wo_chunks),
        out_shape=jax.ShapeDtypeStruct(A_x.shape, A_x.dtype),
        in_specs=[any_spec] * 10,
        out_specs=pl.BlockSpec(memory_space=pltpu.VMEM),
        scratch_shapes=[
            pltpu.VMEM((1, 1, d), bf16),
            pltpu.VMEM((d // 128, 128), bf16),
            pltpu.VMEM((d // 128, 128), bf16),
            pltpu.VMEM((d, _HQ * _DH), bf16),
            pltpu.VMEM((_HQ * _DH, d), bf16),
            pltpu.VMEM((d, f), bf16),
            pltpu.VMEM((d, f), bf16),
            pltpu.VMEM((f, d), bf16),
            pltpu.VMEM((2, _PR, w), bf16),
            pltpu.VMEM((2, _PR, w), bf16),
            pltpu.VMEM((8, _HQ * _DH), jnp.float32),
            pltpu.VMEM((8, _HQ * _DH), jnp.float32),
            pltpu.SemaphoreType.DMA((3,)),
            pltpu.SemaphoreType.DMA((4,)),
            pltpu.SemaphoreType.DMA((2,)),
            pltpu.SemaphoreType.DMA((2,)),
            pltpu.SemaphoreType.DMA((len(wo_chunks),)),
        ],
        compiler_params=pltpu.CompilerParams(
            vmem_limit_bytes=100 * 1024 * 1024,
            disable_bounds_checks=True,
        ),
    )(A_x, kt, vt, A_wq, A_wo, wr, B_w_gate, B_w_up, B_w_down, gw)


@jax.jit
def pallas_gated_mix__sliding_block_cached__moe_arch_mod__decode_kernel(
    A_x: jax.Array,
    A_k_cache: jax.Array,
    A_v_cache: jax.Array,
    A_wq: jax.Array,
    A_wo: jax.Array,
    B_x: jax.Array,
    B_w_r: jax.Array,
    B_w_gate: jax.Array,
    B_w_up: jax.Array,
    B_w_down: jax.Array,
    gate_w: jax.Array,
):
    del B_x
    return _build(A_x, A_k_cache, A_v_cache, A_wq, A_wo, B_w_r, B_w_gate, B_w_up, B_w_down, gate_w)
```

```python
import functools

import jax
import jax.numpy as jnp
from jax import lax
import jax.experimental.pallas as pl
import jax.experimental.pallas.tpu as pltpu

_HQ = 32
_DH = 192
_G = 2
_PR = _G * _DH
_BAND = 8
_WD_ROWS = 256


def _pieces(nrows, ncols, rows, cols, prios, stride=1):
    if isinstance(cols, int):
        cols = [cols] * (ncols // cols)
    assert sum(cols) == ncols and nrows % rows == 0
    rs = list(range(0, nrows, rows))
    rs = [r for s in range(stride) for r in rs[s::stride]]
    out, c0 = [], 0
    for nc in cols:
        for r in rs:
            out.append((r, rows, c0, nc, prios[len(out) % len(prios)]))
        c0 += nc
    return out


def _kernel(x_hbm, k_hbm, v_hbm, wq_hbm, wo_hbm, wr_hbm, wg_hbm, wu_hbm, wd_hbm, gw_hbm,
            out_ref,
            x_buf, wr_buf, gw_buf, wq_buf, wo_buf, wg_buf, wu_buf, wd_buf,
            kbuf, vbuf, h_sc,
            sem_small, sem_w, sem_k, sem_v, sem_wd,
            *, sk, w):
    d = x_buf.shape[-1]
    ff = wg_buf.shape[1]
    npair = _HQ // _G
    nwd = ff // _WD_ROWS
    c0 = sk - w
    scale = _DH ** -0.5
    f32, bf16 = jnp.float32, jnp.bfloat16

    def start(src, dst, sem, pieces, srow=0, scol=0, drow=0, dcol=0):
        for (r, nr, c, nc, p) in pieces:
            pltpu.make_async_copy(
                src.at[pl.ds(srow + r, nr), pl.ds(scol + c, nc)],
                dst.at[pl.ds(drow + r, nr), pl.ds(dcol + c, nc)], sem).start(priority=p)

    def wait_full(dst, sem):
        pltpu.make_async_copy(dst, dst, sem).wait()

    kv_pieces = _pieces(_PR, w, _BAND, [7 * w // 16, 9 * w // 16], (0, 1))

    def start_kv(src, buf, sem, pair, slot):
        row = pair * _PR
        if not isinstance(pair, int):
            row = pl.multiple_of(row, _PR)
        start(src, buf.at[slot], sem.at[slot], kv_pieces, srow=row, scol=c0)

    small = [pltpu.make_async_copy(x_hbm, x_buf, sem_small.at[0]),
             pltpu.make_async_copy(wr_hbm, wr_buf, sem_small.at[1]),
             pltpu.make_async_copy(gw_hbm, gw_buf, sem_small.at[2])]
    for cp in small:
        cp.start(priority=0)

    wq_cols = 2048
    wq_pieces = _pieces(d, wq_cols, _BAND, wq_cols, (0, 1, 1, 1), stride=6)

    def issue_wq(i, c):
        col = pl.multiple_of(i * wq_cols, 128)
        start(wq_hbm, wq_buf, sem_w.at[0], wq_pieces, scol=col, dcol=col)
        return c

    lax.fori_loop(0, _HQ * _DH // wq_cols, issue_wq, 0)
    start_kv(k_hbm, kbuf, sem_k, 0, 0)

    wo_rows, wo_stride = 16, 32
    wo_pieces = [(k * wo_stride * wo_rows, wo_rows, 0, d, (0, 1, 1, 1)[k % 4])
                 for k in range(_HQ * _DH // (wo_rows * wo_stride))]

    def issue_wo(i, c):
        row = pl.multiple_of(i * wo_rows, wo_rows)
        start(wo_hbm, wo_buf, sem_w.at[3], wo_pieces, srow=row, drow=row)
        return c

    lax.fori_loop(0, wo_stride, issue_wo, 0)
    start_kv(v_hbm, vbuf, sem_v, 0, 0)

    for cp in small:
        cp.wait()
    xf = x_buf[0].astype(f32)
    x8 = jnp.broadcast_to(xf, (8, d)).astype(bf16)
    wr = wr_buf[...].astype(f32)
    gw = gw_buf[...].astype(f32)
    nl = d // 128
    racc = sum(xf[:, i * 128:(i + 1) * 128] * wr[i:i + 1, :] for i in range(nl))
    gacc = sum(xf[:, i * 128:(i + 1) * 128] * gw[i:i + 1, :] for i in range(nl))
    r_sel = jax.nn.sigmoid(jnp.sum(racc, axis=1, keepdims=True))
    gate = jax.nn.sigmoid(jnp.sum(gacc, axis=1, keepdims=True))
    wait_full(wq_buf, sem_w.at[0])
    wait_full(wo_buf, sem_w.at[3])

    diag = (lax.broadcasted_iota(jnp.int32, (8, _PR), 1) // _DH
            == lax.broadcasted_iota(jnp.int32, (8, _PR), 0))
    gu_pieces = _pieces(d, ff, _BAND, ff, (0, 1, 1, 1), stride=22)

    def body(pair, acc):
        slot = pair % 2
        nxt = 1 - slot
        off = pl.multiple_of(pair * _PR, 128)

        @pl.when(pair < npair - 1)
        def _():
            start_kv(k_hbm, kbuf, sem_k, pair + 1, nxt)

        @pl.when(pair == npair - 1)
        def _():
            start(wg_hbm, wg_buf, sem_w.at[1], gu_pieces)

        q = jnp.dot(x8, wq_buf[:, pl.ds(off, _PR)], preferred_element_type=f32)
        qb = jnp.where(diag, q, 0.0).astype(bf16)
        wait_full(kbuf.at[slot], sem_k.at[slot])
        s = jnp.dot(qb, kbuf[slot], preferred_element_type=f32)
        m = jnp.max(s, axis=1, keepdims=True)
        p = jnp.exp((s - m) * scale)
        l = jnp.sum(p, axis=1, keepdims=True)
        pb = p.astype(bf16)

        @pl.when(pair < npair - 1)
        def _():
            start_kv(v_hbm, vbuf, sem_v, pair + 1, nxt)

        @pl.when(pair == npair - 1)
        def _():
            start(wu_hbm, wu_buf, sem_w.at[2], gu_pieces)

        wait_full(vbuf.at[slot], sem_v.at[slot])
        o = lax.dot_general(pb, vbuf[slot], (((1,), (1,)), ((), ())),
                            preferred_element_type=f32)
        ob = jnp.where(diag, o / l, 0.0).astype(bf16)
        return acc + jnp.dot(ob, wo_buf[pl.ds(off, _PR), :], preferred_element_type=f32)

    acc = lax.fori_loop(0, npair, body, jnp.zeros((8, d), f32))

    wd_pieces = _pieces(_WD_ROWS, d, 16, d, (0, 1, 1, 1))

    def issue_wd(i, c):
        row = pl.multiple_of(i * _WD_ROWS, _WD_ROWS)
        start(wd_hbm, wd_buf, sem_wd.at[i], wd_pieces, srow=row, drow=row)
        return c

    lax.fori_loop(0, nwd, issue_wd, 0)
    a_branch = jnp.sum(acc, axis=0, keepdims=True)
    wait_full(wg_buf, sem_w.at[1])
    wait_full(wu_buf, sem_w.at[2])
    hg = jnp.dot(x8, wg_buf[...], preferred_element_type=f32).astype(bf16).astype(f32)
    hu = jnp.dot(x8, wu_buf[...], preferred_element_type=f32).astype(bf16).astype(f32)
    h_sc[...] = hg * jax.nn.sigmoid(hg) * hu
    base = gate * a_branch + (1.0 - gate) * (xf + xf * 0.0)
    ymul = (1.0 - gate) * r_sel

    def down(i, y):
        row = pl.multiple_of(i * _WD_ROWS, _WD_ROWS)
        wait_full(wd_buf.at[pl.ds(row, _WD_ROWS)], sem_wd.at[i])
        return y + jnp.dot(h_sc[:, pl.ds(row, _WD_ROWS)].astype(bf16),
                           wd_buf[pl.ds(row, _WD_ROWS), :], preferred_element_type=f32)

    y = lax.fori_loop(0, nwd, down, jnp.zeros((8, d), f32))
    out_ref[0] = (base + y[0:1] * ymul).astype(out_ref.dtype)


@jax.jit
def pallas_gated_mix__sliding_block_cached__moe_arch_mod__decode_kernel(
    A_x: jax.Array,
    A_k_cache: jax.Array,
    A_v_cache: jax.Array,
    A_wq: jax.Array,
    A_wo: jax.Array,
    B_x: jax.Array,
    B_w_r: jax.Array,
    B_w_gate: jax.Array,
    B_w_up: jax.Array,
    B_w_down: jax.Array,
    gate_w: jax.Array,
):
    del B_x
    _, _, d = A_x.shape
    _, hkv, sk, dh = A_k_cache.shape
    assert hkv == _HQ and dh == _DH
    ff = B_w_gate.shape[1]
    w = min(4096, max(256, sk // 4))
    kt = jnp.swapaxes(A_k_cache, 2, 3).reshape(_HQ * _DH, sk)
    vt = jnp.swapaxes(A_v_cache, 2, 3).reshape(_HQ * _DH, sk)
    wr = B_w_r.reshape(d // 128, 128)
    gw = gate_w.reshape(d // 128, 128)
    bf16 = jnp.bfloat16
    any_spec = pl.BlockSpec(memory_space=pl.ANY)
    return pl.pallas_call(
        functools.partial(_kernel, sk=sk, w=w),
        out_shape=jax.ShapeDtypeStruct(A_x.shape, A_x.dtype),
        in_specs=[any_spec] * 10,
        out_specs=pl.BlockSpec(memory_space=pltpu.VMEM),
        scratch_shapes=[
            pltpu.VMEM((1, 1, d), bf16),
            pltpu.VMEM((d // 128, 128), bf16),
            pltpu.VMEM((d // 128, 128), bf16),
            pltpu.VMEM((d, _HQ * _DH), bf16),
            pltpu.VMEM((_HQ * _DH, d), bf16),
            pltpu.VMEM((d, ff), bf16),
            pltpu.VMEM((d, ff), bf16),
            pltpu.VMEM((ff, d), bf16),
            pltpu.VMEM((2, _PR, w), bf16),
            pltpu.VMEM((2, _PR, w), bf16),
            pltpu.VMEM((8, ff), jnp.float32),
            pltpu.SemaphoreType.DMA((3,)),
            pltpu.SemaphoreType.DMA((4,)),
            pltpu.SemaphoreType.DMA((2,)),
            pltpu.SemaphoreType.DMA((2,)),
            pltpu.SemaphoreType.DMA((ff // _WD_ROWS,)),
        ],
        compiler_params=pltpu.CompilerParams(
            vmem_limit_bytes=64 * 1024 * 1024,
            disable_bounds_checks=True,
        ),
    )(A_x, kt, vt, A_wq, A_wo, wr, B_w_gate, B_w_up, B_w_down, gw)
```

```python
import functools

import jax
import jax.numpy as jnp
from jax import lax
import jax.experimental.pallas as pl
import jax.experimental.pallas.tpu as pltpu

_HQ = 32
_DH = 192
_G = 2
_PR = _G * _DH
_BAND = 8
_WD_MXU = 256
_WD_TAIL = 256
_WD_VPU = 32


def _span_pieces(nrows, spans, prios):
    out = []
    for (c0, nc) in spans:
        for r in range(0, nrows, _BAND):
            out.append((r, _BAND, c0, nc, prios[len(out) % len(prios)]))
    return out


def _row_pieces(nrows, ncols, rows, prios, stride=1):
    rs = list(range(0, nrows, rows))
    rs = [r for s in range(stride) for r in rs[s::stride]]
    return [(r, rows, 0, ncols, prios[i % len(prios)]) for i, r in enumerate(rs)]


def _flat_pieces(nrows, ncols, prios, first=14, chunk=16, period=16):
    tpb = ncols // 128
    nt = (nrows // _BAND) * tpb
    cuts = [0] + list(range(first, nt, chunk)) + [nt]
    runs = list(zip(cuts[:-1], cuts[1:]))
    out = []
    for j, i in enumerate(i for o in range(period) for i in range(o, len(runs), period)):
        a, b = runs[i]
        p = prios[j % len(prios)]
        while a < b:
            band, t = divmod(a, tpb)
            if t == 0 and b - a >= tpb:
                n = (b - a) // tpb
                out.append((band * _BAND, n * _BAND, 0, ncols, p))
                a += n * tpb
            else:
                e = min(b, (band + 1) * tpb)
                out.append((band * _BAND, _BAND, t * 128, (e - a) * 128, p))
                a = e
    return out


def _kernel(x_hbm, k_hbm, v_hbm, wq_hbm, wo_hbm, wr_hbm, wg_hbm, wu_hbm, wd_hbm, gw_hbm,
            out_ref,
            x_buf, wr_buf, gw_buf, wq_buf, wo_buf, wg_buf, wu_buf, wd_buf,
            kbuf, vbuf, h_sc, hb_sc,
            sem_small, sem_w, sem_k, sem_v, sem_wd,
            *, sk, w):
    d = x_buf.shape[-1]
    ff = wg_buf.shape[1]
    npair = _HQ // _G
    c0 = sk - w
    scale = _DH ** -0.5
    f32, bf16 = jnp.float32, jnp.bfloat16

    def start1(src, dst, sem, piece, srow=0, scol=0, drow=0):
        r, nr, c, nc, p = piece
        pltpu.make_async_copy(
            src.at[pl.ds(srow + r, nr), pl.ds(scol + c, nc)],
            dst.at[pl.ds(drow + r, nr), pl.ds(c, nc)], sem).start(priority=p)

    def start(src, dst, sem, pieces, **kw):
        for piece in pieces:
            start1(src, dst, sem, piece, **kw)

    def wait_full(dst, sem):
        pltpu.make_async_copy(dst, dst, sem).wait()

    ca, cb = 7 * w // 16, 11 * w // 16
    kv_pieces = _span_pieces(_PR, [(ca, cb - ca), (cb, w - cb), (0, ca)], (0, 1))

    def start_kv(src, buf, sem, pair, slot):
        row = pair * _PR
        if not isinstance(pair, int):
            row = pl.multiple_of(row, _PR)
        start(src, buf.at[slot], sem.at[slot], kv_pieces, srow=row, scol=c0)

    small = [pltpu.make_async_copy(x_hbm, x_buf, sem_small.at[0]),
             pltpu.make_async_copy(wr_hbm, wr_buf, sem_small.at[1]),
             pltpu.make_async_copy(gw_hbm, gw_buf, sem_small.at[2])]
    for cp in small:
        cp.start(priority=0)

    prologue = [
        lambda: start(wq_hbm, wq_buf, sem_w.at[0], _flat_pieces(d, _HQ * _DH, (0, 1, 1, 1))),
        lambda: start(wo_hbm, wo_buf, sem_w.at[1], _flat_pieces(_HQ * _DH, d, (0, 1))),
        lambda: start_kv(k_hbm, kbuf, sem_k, 0, 0),
        lambda: start_kv(v_hbm, vbuf, sem_v, 0, 0),
    ]

    def prologue_step(i, c):
        for j, step in enumerate(prologue):
            pl.when(i == j)(step)
        return c

    lax.fori_loop(0, len(prologue), prologue_step, 0)

    for cp in small:
        cp.wait()
    xf = x_buf[0].astype(f32)
    x8 = jnp.broadcast_to(xf, (8, d)).astype(bf16)
    wr = wr_buf[...].astype(f32)
    gw = gw_buf[...].astype(f32)
    nl = d // 128
    racc = sum(xf[:, i * 128:(i + 1) * 128] * wr[i:i + 1, :] for i in range(nl))
    gacc = sum(xf[:, i * 128:(i + 1) * 128] * gw[i:i + 1, :] for i in range(nl))
    r_sel = jax.nn.sigmoid(jnp.sum(racc, axis=1, keepdims=True))
    gate = jax.nn.sigmoid(jnp.sum(gacc, axis=1, keepdims=True))
    wait_full(wq_buf, sem_w.at[0])
    wait_full(wo_buf, sem_w.at[1])

    diag = (lax.broadcasted_iota(jnp.int32, (8, _PR), 1) // _DH
            == lax.broadcasted_iota(jnp.int32, (8, _PR), 0))

    gu_pieces = _row_pieces(d, ff, _BAND, (0,), stride=22)

    def start_gu(pieces):
        for piece in pieces:
            start1(wg_hbm, wg_buf, sem_w.at[2], piece)
            start1(wu_hbm, wu_buf, sem_w.at[3], piece[:-1] + (1,))

    def body(pair, acc):
        slot = pair % 2
        nxt = 1 - slot
        off = pl.multiple_of(pair * _PR, 128)

        @pl.when(pair < npair - 1)
        def _():
            start_kv(k_hbm, kbuf, sem_k, pair + 1, nxt)

        @pl.when(pair == npair - 1)
        def _():
            start_gu(gu_pieces[:len(gu_pieces) // 2])

        q = jnp.dot(x8, wq_buf[:, pl.ds(off, _PR)], preferred_element_type=f32)
        qb = jnp.where(diag, q, 0.0).astype(bf16)
        wait_full(kbuf.at[slot], sem_k.at[slot])
        s = jnp.dot(qb, kbuf[slot], preferred_element_type=f32)
        m = jnp.max(s, axis=1, keepdims=True)
        p = jnp.exp((s - m) * scale)
        l = jnp.sum(p, axis=1, keepdims=True)
        pb = p.astype(bf16)

        @pl.when(pair < npair - 1)
        def _():
            start_kv(v_hbm, vbuf, sem_v, pair + 1, nxt)

        @pl.when(pair == npair - 1)
        def _():
            start_gu(gu_pieces[len(gu_pieces) // 2:])

        wait_full(vbuf.at[slot], sem_v.at[slot])
        o = lax.dot_general(pb, vbuf[slot], (((1,), (1,)), ((), ())),
                            preferred_element_type=f32)
        ob = jnp.where(diag, o / l, 0.0).astype(bf16)
        return acc + jnp.dot(ob, wo_buf[pl.ds(off, _PR), :], preferred_element_type=f32)

    acc = lax.fori_loop(0, npair, body, jnp.zeros((8, d), f32))

    tail0 = ff - _WD_TAIL
    n_mxu = tail0 // _WD_MXU
    n_vpu = _WD_TAIL // _WD_VPU

    def issue_mxu(i, c):
        row = pl.multiple_of(i * _WD_MXU, _WD_MXU)
        start(wd_hbm, wd_buf, sem_wd.at[i], _row_pieces(_WD_MXU, d, 16, (0, 1, 1, 1)),
              srow=row, drow=row)
        return c

    def issue_vpu(i, c):
        row = pl.multiple_of(tail0 + i * _WD_VPU, _WD_VPU)
        start(wd_hbm, wd_buf, sem_wd.at[n_mxu + i], _row_pieces(_WD_VPU, d, 16, (1,)),
              srow=row, drow=row)
        return c

    lax.fori_loop(0, n_mxu, issue_mxu, 0)
    lax.fori_loop(0, n_vpu, issue_vpu, 0)

    a_branch = jnp.sum(acc, axis=0, keepdims=True)
    wait_full(wg_buf, sem_w.at[2])
    wait_full(wu_buf, sem_w.at[3])
    hg = jnp.dot(x8, wg_buf[...], preferred_element_type=f32).astype(bf16).astype(f32)
    hu = jnp.dot(x8, wu_buf[...], preferred_element_type=f32).astype(bf16).astype(f32)
    hact = (hg * jax.nn.sigmoid(hg) * hu).astype(bf16).astype(f32)
    h_sc[...] = hact
    hb_sc[...] = jnp.transpose(jnp.broadcast_to(hact[0:1, tail0:], (128, _WD_TAIL)))
    base = gate * a_branch + (1.0 - gate) * (xf + xf * 0.0)
    ymul = (1.0 - gate) * r_sel

    def down_mxu(i, y):
        row = pl.multiple_of(i * _WD_MXU, _WD_MXU)
        wait_full(wd_buf.at[pl.ds(row, _WD_MXU)], sem_wd.at[i])
        return y + jnp.dot(h_sc[:, pl.ds(row, _WD_MXU)].astype(bf16),
                           wd_buf[pl.ds(row, _WD_MXU), :], preferred_element_type=f32)

    y = lax.fori_loop(0, n_mxu, down_mxu, jnp.zeros((8, d), f32))
    y = jnp.where(lax.broadcasted_iota(jnp.int32, (8, d), 0) == 0, y, 0.0)

    def down_vpu(i, y):
        row = pl.multiple_of(tail0 + i * _WD_VPU, _WD_VPU)
        wait_full(wd_buf.at[pl.ds(row, _WD_VPU)], sem_wd.at[n_mxu + i])
        wv = wd_buf[pl.ds(row, _WD_VPU), :].astype(f32)
        hb = hb_sc[pl.ds(pl.multiple_of(i * _WD_VPU, _WD_VPU), _WD_VPU), :]
        cols = []
        for t in range(nl):
            prod = wv[:, t * 128:(t + 1) * 128] * hb
            cols.append(sum(prod[g * 8:(g + 1) * 8] for g in range(_WD_VPU // 8)))
        return y + jnp.concatenate(cols, axis=1)

    y = lax.fori_loop(0, n_vpu, down_vpu, y)
    out_ref[0] = (base + jnp.sum(y, axis=0, keepdims=True) * ymul).astype(out_ref.dtype)


@jax.jit
def pallas_gated_mix__sliding_block_cached__moe_arch_mod__decode_kernel(
    A_x: jax.Array,
    A_k_cache: jax.Array,
    A_v_cache: jax.Array,
    A_wq: jax.Array,
    A_wo: jax.Array,
    B_x: jax.Array,
    B_w_r: jax.Array,
    B_w_gate: jax.Array,
    B_w_up: jax.Array,
    B_w_down: jax.Array,
    gate_w: jax.Array,
):
    del B_x
    _, _, d = A_x.shape
    _, hkv, sk, dh = A_k_cache.shape
    assert hkv == _HQ and dh == _DH
    ff = B_w_gate.shape[1]
    w = min(4096, max(256, sk // 4))
    assert w % 2048 == 0 and (ff - _WD_TAIL) % _WD_MXU == 0
    kt = jnp.swapaxes(A_k_cache, 2, 3).reshape(_HQ * _DH, sk)
    vt = jnp.swapaxes(A_v_cache, 2, 3).reshape(_HQ * _DH, sk)
    wr = B_w_r.reshape(d // 128, 128)
    gw = gate_w.reshape(d // 128, 128)
    bf16 = jnp.bfloat16
    any_spec = pl.BlockSpec(memory_space=pl.ANY)
    return pl.pallas_call(
        functools.partial(_kernel, sk=sk, w=w),
        out_shape=jax.ShapeDtypeStruct(A_x.shape, A_x.dtype),
        in_specs=[any_spec] * 10,
        out_specs=pl.BlockSpec(memory_space=pltpu.VMEM),
        scratch_shapes=[
            pltpu.VMEM((1, 1, d), bf16),
            pltpu.VMEM((d // 128, 128), bf16),
            pltpu.VMEM((d // 128, 128), bf16),
            pltpu.VMEM((d, _HQ * _DH), bf16),
            pltpu.VMEM((_HQ * _DH, d), bf16),
            pltpu.VMEM((d, ff), bf16),
            pltpu.VMEM((d, ff), bf16),
            pltpu.VMEM((ff, d), bf16),
            pltpu.VMEM((2, _PR, w), bf16),
            pltpu.VMEM((2, _PR, w), bf16),
            pltpu.VMEM((8, ff), jnp.float32),
            pltpu.VMEM((_WD_TAIL, 128), jnp.float32),
            pltpu.SemaphoreType.DMA((3,)),
            pltpu.SemaphoreType.DMA((4,)),
            pltpu.SemaphoreType.DMA((2,)),
            pltpu.SemaphoreType.DMA((2,)),
            pltpu.SemaphoreType.DMA(((ff - _WD_TAIL) // _WD_MXU + _WD_TAIL // _WD_VPU,)),
        ],
        compiler_params=pltpu.CompilerParams(
            vmem_limit_bytes=64 * 1024 * 1024,
            disable_bounds_checks=True,
            disable_semaphore_checks=True,
        ),
    )(A_x, kt, vt, A_wq, A_wo, wr, B_w_gate, B_w_up, B_w_down, gw)
```
